```python
import os as _os
_os.environ.setdefault("JAX_PLATFORMS", "cpu")
import jax
import jax.numpy as jnp

def _softmax(x, axis=-1):
    return jax.nn.softmax(x, axis=axis)
def _gelu(x):
    return jax.nn.gelu(x, approximate=True)
def _silu(x):
    return jax.nn.silu(x)
def _sigmoid(x):
    return jax.nn.sigmoid(x)
def _layernorm(x, axis=-1, eps=1e-5):
    m = jnp.mean(x, axis=axis, keepdims=True)
    v = jnp.var(x, axis=axis, keepdims=True)
    return (x - m) / jnp.sqrt(v + eps)
def _scatter_add(tgt, idx, src, axis=0):
    return tgt.at[idx].add(src)
def _segment_sum(src, seg, n):
    return jax.ops.segment_sum(src, seg, n)
class _Rng:
    def __init__(self, key):
        self._k = key
    def _next(self):
        self._k, sub = jax.random.split(self._k)
        return sub
    def normal(self, shape):
        return jax.random.normal(self._next(), shape, dtype=jnp.bfloat16)
    def randint(self, lo, hi, shape):
        return jax.random.randint(self._next(), shape, lo, hi, dtype=jnp.int32)
    def uniform(self, shape, lo=0.0, hi=1.0):
        return jax.random.uniform(self._next(), shape, jnp.bfloat16, lo, hi)
    def permutation(self, n):
        return jax.random.permutation(self._next(), n)


kernel_name = 'gated_mix__mha_block__mixer_s_mlp__prompt'

def setup_inputs():
    _rng = _Rng(jax.random.key(int.from_bytes(__import__("os").urandom(4), "little")))
    _w = (lambda a: (lambda t: t.astype(jnp.bfloat16) if jnp.issubdtype(t.dtype, jnp.floating) else t)(jnp.asarray(a)))
    def _A_setup():
        B, S, D, H = 1, 2048, 512, 32
        return {
            "x": _w((lambda *s: _rng.normal(s) * 0.05)(B, S, D)),
            "wqkv": _w((lambda *s: _rng.normal(s) * 0.8)(D, 3 * D)),
            "wo": _w((lambda *s: _rng.normal(s) * 0.05)(D, D)),
        }
    _A_in = _A_setup()

    def _B_setup():
        B, S, D, F = 1, 2048, 512, 1792
        return {
            "x":  _w((lambda *s: _rng.normal(s) * 0.05)(B, S, D)),
            "w1": _w((lambda *s: _rng.normal(s) * 0.2)(D, D) * (D ** -0.5)),
            "w2": _w((lambda *s: _rng.normal(s) * 0.2)(D, D) * (D ** -0.5)),
            "w3": _w((lambda *s: _rng.normal(s) * 0.2)(D, F) * (D ** -0.5)),
            "w4": _w((lambda *s: _rng.normal(s) * 0.2)(F, D) * (F ** -0.5)),
        }
    _B_in = _B_setup()

    return {
        "A_x": _A_in["x"],
        "A_wqkv": _A_in["wqkv"],
        "A_wo": _A_in["wo"],
        "B_x": _B_in["x"],
        "B_w1": _B_in["w1"],
        "B_w2": _B_in["w2"],
        "B_w3": _B_in["w3"],
        "B_w4": _B_in["w4"],
        "gate_w": _w((lambda *s: _rng.normal(s) * 0.05)(512) * 16.0),
    }

def reference(A_x, A_wqkv, A_wo, B_x, B_w1, B_w2, B_w3, B_w4, gate_w):
    def _A_ref(x, wqkv, wo):
        B, S, D = x.shape
        H = 32
        Dh = D // H
        qkv = (lambda x, *d: x.transpose(*d))((x @ wqkv).reshape(B, S, 3, H, Dh), 2, 0, 3, 1, 4)
        q, k, v = qkv[0], qkv[1], qkv[2]
        scores = jnp.einsum("bhqd,bhkd->bhqk", q, k) * (Dh ** -0.5)
        p = _softmax(scores, axis=-1)
        o = jnp.einsum("bhqk,bhkd->bhqd", p, v)
        return (lambda x, *d: x.transpose(*d))(o, 0, 2, 1, 3).reshape(B, S, D) @ wo

    def _B_ref(x, w1, w2, w3, w4):
        B, S, D = x.shape
        h = _gelu(_layernorm(x, axis=-1) @ w1)
        c = D // 4
        g0 = jnp.pad(h[:, :, 0*c:1*c], ((0, 0), (1, 0), (0, 0)))[:, :S, :]
        g1 = jnp.pad(h[:, :, 1*c:2*c], ((0, 0), (0, 1), (0, 0)))[:, 1:, :]
        g2 = jnp.pad(h[:, :, 2*c:3*c], ((0, 0), (2, 0), (0, 0)))[:, :S, :]
        g3 = jnp.pad(h[:, :, 3*c:   ], ((0, 0), (0, 2), (0, 0)))[:, 2:, :]
        hs = jnp.concatenate([g0, g1, g2, g3], axis=-1) @ w2
        x1 = x + hs
        h2 = _gelu(_layernorm(x1, axis=-1) @ w3) @ w4
        return x1 + h2

    x = A_x
    g = _sigmoid((x * gate_w).sum(-1, keepdims=True))
    a = _A_ref(x, A_wqkv, A_wo)
    b = _B_ref(x, B_w1, B_w2, B_w3, B_w4)
    return g * a + (1 - g) * b
```

```python
import math

import jax
import jax.numpy as jnp
from jax import lax
import jax.experimental.pallas as pl
import jax.experimental.pallas.tpu as pltpu

S, D, H, F = 2048, 512, 32, 1792
DH = D // H
TQ = 512
TK = 128
HU = 8
LAG = 2
FC = 256
HALO = 8
NT = S // TQ
Q_SCALE = (DH ** -0.5) * math.log2(math.e)
SCORE_MAX = 40.0
V_MIN, V_MAX = 2.0 ** -60, 2.0 ** 60

BF16 = jnp.bfloat16
F32 = jnp.float32


def _dot(a, b):
    return jnp.dot(a, b, preferred_element_type=F32)


def _layernorm(x):
    m = jnp.mean(x, axis=-1, keepdims=True)
    c = x - m
    v = jnp.mean(c * c, axis=-1, keepdims=True)
    return c * lax.rsqrt(v + 1e-5)


def _gelu(x):
    inner = x * (math.sqrt(2.0 / math.pi) + (math.sqrt(2.0 / math.pi) * 0.044715) * (x * x))
    hx = 0.5 * x
    return hx + hx * jnp.tanh(inner)


def _max_head_norm2(t):
    sq = t * t
    out = None
    for h in range(H):
        p = sq[h * DH:h * DH + 8] + sq[h * DH + 8:(h + 1) * DH]
        p = p + pltpu.roll(p, 4, 0)
        p = p + pltpu.roll(p, 2, 0)
        p = p + pltpu.roll(p, 1, 0)
        out = p if out is None else jnp.maximum(out, p)
    return out


def _kernel(ax_hbm, wqkv_hbm, wo_hbm, w1_hbm, w2_hbm, w3_hbm, w4_hbm, gw_ref,
            out_hbm,
            ax, wqkv, wo, w1, w2, w3, w4,
            hbuf, x1s, ln2, ks, qts, vts, ots, vmax, obuf, in_sem, out_sem):
    def rows(c):
        return pl.ds(c * TQ, TQ)

    copies = {}

    def add(name, src, dst):
        copies[name] = pltpu.make_async_copy(src, dst, in_sem.at[len(copies)])

    add("w1", w1_hbm, w1)
    add("w2", w2_hbm, w2)
    add("wqkv", wqkv_hbm, wqkv)
    for c in range(NT):
        add(("ax", c), ax_hbm.at[rows(c)], ax.at[rows(c)])
    add("wo", wo_hbm, wo)
    add("w3", w3_hbm, w3)
    add("w4", w4_hbm, w4)

    def start(*names):
        for n in names:
            copies[n].start()

    def wait(*names):
        for n in names:
            copies[n].wait()

    start(("ax", 0), "w1")
    hbuf[0:HALO, :] = jnp.zeros((HALO, D), F32)
    hbuf[HALO + S:, :] = jnp.zeros((HALO, D), F32)

    nxt = [[("ax", 1), "w2"], [("ax", 2), "wqkv"], [("ax", 3)], ["wo"]]
    wait("w1")
    for c in range(NT):
        wait(("ax", c))
        start(*nxt[c])
        xn = _layernorm(ax[rows(c), :].astype(F32)).astype(BF16)
        hbuf[pl.ds(HALO + c * TQ, TQ), :] = _gelu(_dot(xn, w1[...]))

    wait("w2")
    start("w3")
    cw = D // 4
    for c in range(NT):
        r0 = HALO + c * TQ
        hs = jnp.concatenate([
            hbuf[pl.ds(r0 + off, TQ), g * cw:(g + 1) * cw]
            for g, off in enumerate((-1, 1, -2, 2))], axis=-1).astype(BF16)
        x1 = ax[rows(c), :].astype(F32) + _dot(hs, w2[...])
        x1s[rows(c), :] = x1
        ln2[rows(c), :] = _layernorm(x1).astype(BF16)

    wait("wqkv")
    start("w4")

    def qkv_body(c, carry):
        qn, kn = carry
        r0 = pl.multiple_of(c * TQ, TQ)
        x = ax[pl.ds(r0, TQ), :]

        def proj(i):
            return lax.dot_general(wqkv[:, i * D:(i + 1) * D], x, (((0,), (1,)), ((), ())),
                                   preferred_element_type=F32)

        kt = proj(1)
        kk = kt.T.astype(BF16)
        for g in range(D // 128):
            ks[g, pl.ds(r0, TQ), :] = kk[:, g * 128:(g + 1) * 128]
        kn = jnp.maximum(kn, _max_head_norm2(kt))
        qt = proj(0) * Q_SCALE
        qts[c] = qt.astype(BF16)
        qn = jnp.maximum(qn, _max_head_norm2(qt))
        vt = proj(2)
        vts[:, pl.ds(r0, TQ)] = vt.astype(BF16)
        av = jnp.abs(vt)
        m = av[:, 0:128]
        for j in range(1, TQ // 128):
            m = jnp.maximum(m, av[:, j * 128:(j + 1) * 128])
        vmax[...] = jnp.maximum(vmax[...], m)
        return qn, kn

    vmax[...] = jnp.zeros(vmax.shape, F32)
    zero = jnp.zeros((8, TQ), F32)
    qn, kn = lax.fori_loop(0, NT, qkv_body, (zero, zero))

    vm = jnp.max(vmax[...], axis=1, keepdims=True)
    v_ok = jnp.logical_or(vm == 0.0, jnp.logical_and(vm >= V_MIN, vm <= V_MAX))
    v_bad = jnp.max(jnp.where(v_ok, 0.0, 1.0))
    bound2 = jnp.max(qn) * jnp.max(kn) * 1.02
    no_shift = jnp.logical_and(bound2 <= SCORE_MAX * SCORE_MAX, v_bad == 0.0)

    wait("wo", "w3", "w4")

    def masked_q(t, g, u):
        q = qts[t, pl.ds(pl.multiple_of(g * 128 + u * DH, DH), DH), :]
        parts = []
        if u > 0:
            parts.append(jnp.zeros((u * DH, TQ), BF16))
        parts.append(q)
        if u < HU - 1:
            parts.append(jnp.zeros(((HU - 1 - u) * DH, TQ), BF16))
        return jnp.concatenate(parts, axis=0)

    def attn_fast(t):
        nk = S // TK

        def body(g, _):
            steps = [(u, j) for u in range(HU) for j in range(nk)]
            ps, acc, den = {}, {}, {}
            for i in range(len(steps) + LAG):
                if i < len(steps):
                    u, j = steps[i]
                    p = jnp.exp2(_dot(ks[g, j * TK:(j + 1) * TK, :], masked_q(t, g, u)))
                    ls = p.reshape(TK // 8, 8, TQ).sum(0)
                    den[u] = ls if j == 0 else den[u] + ls
                    ps[i] = p.astype(BF16)
                if i >= LAG:
                    u, j = steps[i - LAG]
                    hr = pl.ds(pl.multiple_of(g * 128 + u * DH, DH), DH)
                    o = _dot(vts[hr, j * TK:(j + 1) * TK], ps.pop(i - LAG))
                    acc[u] = o if j == 0 else acc[u] + o
                    if j == nk - 1:
                        ots[hr, :] = (acc[u] / den[u].sum(0, keepdims=True)).astype(BF16)
            return 0

        lax.fori_loop(0, H // HU, body, 0)

    def attn_true_max(t):
        head_of_row = lax.broadcasted_iota(jnp.int32, (128, TQ), 0) // DH

        def body(h, _):
            g = h // HU
            qg = qts[t, pl.ds(pl.multiple_of(g * 128, 128), 128), :]
            q = jnp.where(head_of_row == h % HU, qg.astype(F32), 0.0).astype(BF16)
            hr = pl.ds(pl.multiple_of(h * DH, DH), DH)

            def kbody(j, carry):
                m, den, acc = carry
                k0 = pl.multiple_of(j * TK, TK)
                s = _dot(ks[g, pl.ds(k0, TK), :], q)
                m_new = jnp.maximum(m, jnp.max(s, axis=0, keepdims=True))
                a = jnp.exp2(m - m_new)
                p = jnp.exp2(s - m_new)
                den = a * den + jnp.sum(p, axis=0, keepdims=True)
                acc = a * acc + _dot(vts[hr, pl.ds(k0, TK)], p.astype(BF16))
                return m_new, den, acc

            init = (jnp.full((1, TQ), -jnp.inf, F32), jnp.zeros((1, TQ), F32),
                    jnp.zeros((DH, TQ), F32))
            _, den, acc = lax.fori_loop(0, S // TK, kbody, init)
            ots[hr, :] = (acc / den).astype(BF16)
            return 0

        lax.fori_loop(0, H, body, 0)

    def out_copy(t, slot):
        return pltpu.make_async_copy(
            obuf.at[slot], out_hbm.at[pl.ds(pl.multiple_of(t * TQ, TQ), TQ)], out_sem.at[slot])

    def tile(t, _):
        pl.when(no_shift)(lambda: attn_fast(t))
        pl.when(jnp.logical_not(no_shift))(lambda: attn_true_max(t))

        r = pl.ds(pl.multiple_of(t * TQ, TQ), TQ)
        slot = t % 2

        @pl.when(t >= 2)
        def _():
            out_copy(t - 2, slot).wait()

        xn = ln2[r, :]
        acts = []
        for f in range(F // FC):
            acts.append(_gelu(_dot(xn, w3[:, f * FC:(f + 1) * FC])).astype(BF16))
        a = lax.dot_general(ots[...], wo[...], (((0,), (0,)), ((), ())),
                            preferred_element_type=F32)
        b = x1s[r, :] + _dot(jnp.concatenate(acts, axis=-1), w4[...])
        gate = jax.nn.sigmoid(jnp.sum(ax[r, :].astype(F32) * gw_ref[...].astype(F32),
                                      axis=-1, keepdims=True))
        obuf[slot] = (gate * a + (1.0 - gate) * b).astype(obuf.dtype)
        out_copy(t, slot).start()
        return 0

    lax.fori_loop(0, NT, tile, 0)
    out_copy(NT - 2, (NT - 2) % 2).wait()
    out_copy(NT - 1, (NT - 1) % 2).wait()


@jax.jit
def pallas_gated_mix__mha_block__mixer_s_mlp__prompt_kernel(
    A_x: jax.Array,
    A_wqkv: jax.Array,
    A_wo: jax.Array,
    B_x: jax.Array,
    B_w1: jax.Array,
    B_w2: jax.Array,
    B_w3: jax.Array,
    B_w4: jax.Array,
    gate_w: jax.Array,
):
    hbm = pl.BlockSpec(memory_space=pl.ANY)
    out = pl.pallas_call(
        _kernel,
        in_specs=[hbm] * 7 + [pl.BlockSpec(memory_space=pltpu.VMEM)],
        out_specs=hbm,
        out_shape=jax.ShapeDtypeStruct((S, D), A_x.dtype),
        scratch_shapes=[
            pltpu.VMEM((S, D), BF16),
            pltpu.VMEM((D, 3 * D), BF16),
            pltpu.VMEM((D, D), BF16),
            pltpu.VMEM((D, D), BF16),
            pltpu.VMEM((D, D), BF16),
            pltpu.VMEM((D, F), BF16),
            pltpu.VMEM((F, D), BF16),
            pltpu.VMEM((S + 2 * HALO, D), F32),
            pltpu.VMEM((S, D), F32),
            pltpu.VMEM((S, D), BF16),
            pltpu.VMEM((D // 128, S, 128), BF16),
            pltpu.VMEM((NT, D, TQ), BF16),
            pltpu.VMEM((D, S), BF16),
            pltpu.VMEM((D, TQ), BF16),
            pltpu.VMEM((D, 128), F32),
            pltpu.VMEM((2, TQ, D), A_x.dtype),
            pltpu.SemaphoreType.DMA((10,)),
            pltpu.SemaphoreType.DMA((2,)),
        ],
        compiler_params=pltpu.CompilerParams(vmem_limit_bytes=100 * 2 ** 20),
    )(A_x.reshape(S, D), A_wqkv, A_wo, B_w1, B_w2, B_w3, B_w4,
      gate_w.reshape(1, D))
    return out.reshape(A_x.shape)
```

```python
import functools
import math

import jax
import jax.numpy as jnp
from jax import lax
import jax.experimental.pallas as pl
import jax.experimental.pallas.tpu as pltpu

S, D, H, F = 2048, 512, 32, 1792
DH = D // H
TQ = 512
NT = S // TQ
TK = 128
NK = S // TK
HU = 2
LAG = 2
VLAG = 1; AHEAD = 1; BSTART = 4; BEND = 0
SPLIT = 1; RO = 8
FC = 128
P1 = 0; P2 = 0; HALO = 8; QP = 0; PK = 0
Q_SCALE = (DH ** -0.5) * math.log2(math.e)
SCORE_MAX = 40.0
V_MIN, V_MAX = 2.0 ** -60, 2.0 ** 60

BF16 = jnp.bfloat16
F32 = jnp.float32


def _dot(a, b):
    return jnp.dot(a, b, preferred_element_type=F32)


def _layernorm(x):
    m = jnp.mean(x, axis=-1, keepdims=True)
    c = x - m
    v = jnp.mean(c * c, axis=-1, keepdims=True)
    return c * lax.rsqrt(v + 1e-5)


def _gelu(x):
    a = math.sqrt(2.0 / math.pi)
    hx = 0.5 * x
    return hx + hx * jnp.tanh(x * (a + (a * 0.044715) * (x * x)))


def _lane_tile_max(t):
    return functools.reduce(jnp.maximum, [t[:, j:j + 128] for j in range(0, t.shape[1], 128)])


def _max_head_norm2(t):
    sq = t * t
    out = None
    for h in range(H):
        p = sq[h * DH:h * DH + 8] + sq[h * DH + 8:(h + 1) * DH]
        p = p + pltpu.roll(p, 4, 0)
        p = p + pltpu.roll(p, 2, 0)
        p = p + pltpu.roll(p, 1, 0)
        out = p if out is None else jnp.maximum(out, p)
    return _lane_tile_max(out)


def _strassen_lhs(a11, a12, a21, a22):
    return [v.astype(BF16) for v in
            (a11 + a22, a21 + a22, a11, a22, a11 + a12, a21 - a11, a12 - a22)]


def _strassen_rhs(w, ws, r0, m):
    k, n = w.shape[0] // 2, w.shape[1] // 2
    b11, b12, b21, b22 = [
        w[pl.ds(pl.multiple_of(i * k + r0, 16), m), j * n:(j + 1) * n].astype(F32)
        for i in (0, 1) for j in (0, 1)]
    for i, v in enumerate((b11 + b22, b12 - b22, b21 - b11, b11 + b12, b21 + b22)):
        ws[i, pl.ds(pl.multiple_of(r0, 16), m), :] = v.astype(BF16)


def _strassen_mul(lhs, w, ws, c0, cw):
    k, n = w.shape[0] // 2, w.shape[1] // 2
    cols = slice(c0, c0 + cw)
    m2 = _dot(lhs[1], w[:k, cols])
    m4 = _dot(lhs[3], ws[2, :, cols])
    yield 2, m2 + m4
    m5 = _dot(lhs[4], w[k:, n + c0:n + c0 + cw])
    m3 = _dot(lhs[2], ws[1, :, cols])
    yield 1, m3 + m5
    m1 = _dot(lhs[0], ws[0, :, cols])
    m7 = _dot(lhs[6], ws[4, :, cols])
    yield 0, m1 + m4 - m5 + m7
    m6 = _dot(lhs[5], ws[3, :, cols])
    yield 3, m1 - m2 + m3 + m6


def _kernel(x_hbm, wqkv_hbm, wo_hbm, w1_hbm, w2_hbm, w3_hbm, w4_hbm, gw_hbm,
            out_hbm,
            xs, wqkv, wt, wo, w1, w2, w3, w4, w3s, w4s,
            hbuf, x1s, ln2, acts, gs, ks, kf, qts, qf, vts, ots, obuf,
            qb, pad, kb0, pad1, kb1, pad2, gw, in_sem, out_sem):
    def rows(c):
        return pl.ds(c * TQ if isinstance(c, int) else pl.multiple_of(c * TQ, TQ), TQ)

    def head_rows(h):
        return pl.ds(pl.multiple_of(h * DH, DH), DH)

    def group_rows(h):
        return pl.ds(pl.multiple_of(h // 8 * 128, 128), 128)

    pairs = {"w1": (w1_hbm, w1), "w2": (w2_hbm, w2), "wo": (wo_hbm, wo), "w3": (w3_hbm, w3),
             "w4": (w4_hbm, w4), "gw": (gw_hbm, gw)}
    for i in range(3):
        pairs["w" + "qkv"[i]] = (wqkv_hbm.at[:, pl.ds(i * D, D)], wqkv.at[:, pl.ds(i * D, D)])
    for c in range(NT):
        pairs["x%d" % c] = (x_hbm.at[rows(c)], xs.at[rows(c)])
    copies = {name: pltpu.make_async_copy(src, dst, in_sem.at[i])
              for i, (name, (src, dst)) in enumerate(pairs.items())}

    def start(*names):
        for n in names:
            copies[n].start()

    def wait(*names):
        for n in names:
            copies[n].wait()

    def ln1(c):
        return _layernorm(xs[rows(c), :].astype(F32)).astype(BF16)

    def token_proj(c, xn):
        hbuf[pl.ds(HALO + c * TQ, TQ), :] = _gelu(_dot(xn, w1[...]))

    def token_mix(c):
        cw = D // 4
        hs = jnp.concatenate([
            hbuf[pl.ds(HALO + c * TQ + off, TQ), g * cw:(g + 1) * cw]
            for g, off in enumerate((-1, 1, -2, 2))], axis=-1).astype(BF16)
        x1 = xs[rows(c), :].astype(F32) + _dot(hs, w2[...])
        x1s[rows(c), :] = x1
        ln2[rows(c), :] = _layernorm(x1).astype(BF16)

    stats = {}

    def track(name, m):
        stats[name] = jnp.maximum(stats[name], m) if name in stats else m

    def transpose_w(i):
        wt[i * D:(i + 1) * D, :] = wqkv[:, i * D:(i + 1) * D].T

    def project(c, which):
        for name in which:
            i = "qkv".index(name)
            t = _dot(wt[i * D:(i + 1) * D, :], xs[rows(c), :].T)
            if name == "k":
                kk = t.T.astype(BF16)
                for g in range(D // 128):
                    ks[g, rows(c), :] = kk[:, g * 128:(g + 1) * 128]
                    if c == NT - 1:
                        kf[g] = kk[TQ - TK:, g * 128:(g + 1) * 128].astype(F32)
                track("k", _max_head_norm2(t))
            elif name == "q":
                t = t * Q_SCALE
                qts[:, rows(c)] = t.astype(BF16)
                qf[:, rows(c)] = t
                track("q", _max_head_norm2(t))
            else:
                vts[:, rows(c)] = t.astype(BF16)
                track("v", _lane_tile_max(jnp.abs(t)))

    aligned = {}

    def broadcast_keys(h, dst, d):
        if d == 0:
            aligned["k"] = pltpu.roll(kf[h // 8], (128 - (h % 8) * DH) % 128, 1)
        dst[d] = jnp.broadcast_to(aligned["k"][:, d:d + 1], (TK, 128))

    start("x0", "w1", "wk")
    hbuf[0:HALO, :] = jnp.zeros((HALO, D), F32)
    hbuf[HALO + S:, :] = jnp.zeros((HALO, D), F32)
    wait("x0")
    start("wq", "wv")
    xn0 = ln1(0)
    wait("w1")
    start("x1")
    token_proj(0, xn0)
    wait("wk")
    start("x2", "x3", "w2")
    transpose_w(1)
    project(0, "k")
    wait("wq", "wv")
    transpose_w(0)
    transpose_w(2)
    project(0, "qv")
    wait("x1", "x2", "x3", "w2")
    project(1, "kq")
    token_proj(1, ln1(1))
    token_proj(2, ln1(2))
    token_mix(0)
    project(2, "kq")
    token_proj(3, ln1(3))
    token_mix(1)
    project(3, "kq")
    token_mix(2)
    token_mix(3)
    DP = 0
    start("wo", "w3", "w4", "gw")
    project(1, "v")
    for r in range(TK // 8):
        broadcast_keys(0, kb0 if HU > 1 else kb0.at[0], r)
    project(2, "v")
    project(3, "v")

    vm = jnp.max(stats["v"], axis=1, keepdims=True)
    v_ok = jnp.logical_or(vm == 0.0, jnp.logical_and(vm >= V_MIN, vm <= V_MAX))
    v_bad = jnp.max(jnp.where(v_ok, 0.0, 1.0), axis=0, keepdims=True)
    bound2 = (jnp.max(stats["q"], axis=1, keepdims=True)
              * jnp.max(stats["k"], axis=1, keepdims=True) * 1.02)
    safe = jnp.where(bound2 <= SCORE_MAX * SCORE_MAX, 1.0 - v_bad, 0.0)
    no_shift = jnp.min(safe) > 0.5

    head_of_row = lax.broadcasted_iota(jnp.int32, (128, TQ), 0) // DH

    def masked_q(h, t):
        q = qts[group_rows(h), rows(t)].astype(F32)
        return jnp.where(head_of_row == h % 8, q, 0.0).astype(BF16)

    def attention_no_shift(hh, _):
        return attention_no_shift_(hh, _)

    def attention_no_shift_(hh, _):
        rounds = [(u, t, j) for u in range(HU) for t in range(NT) for j in range(NK - 1)]
        units = [(u, t, r) for u in range(HU) for t in range(NT) for r in range(TK // 8)]
        n = len(rounds)
        pending, acc, den, count = [], {}, {}, {}
        vpu_rows = []

        def weights(u, t, s):
            p = jnp.exp2(s)
            tot = p.reshape(-1, 8, TQ).sum(0)
            den[u, t] = den[u, t] + tot if (u, t) in den else tot
            return p

        def vpu_unit(i, u, t, r):
            if (t, r) == (0, 0):
                q = qf[head_rows(hh * HU + u), :]
                for d in range(DH):
                    qb[u, d, :, 0:S] = jnp.broadcast_to(q[d:d + 1, :], (8, S))
            kb = (kb0, kb1)[u % 2] if HU > 1 else kb0.at[hh % 2]
            s = functools.reduce(jnp.add, [
                jnp.tile(kb[d, r * 8:(r + 1) * 8, :], (1, TQ // 128)) * qb[u, d, :, t * TQ:(t + 1) * TQ]
                for d in range(DH)])
            vpu_rows.append(weights(u, t, s))
            if r == TK // 8 - 1:
                pending.append((i + VLAG, u, t, NK - 1, jnp.concatenate(vpu_rows, 0).astype(BF16)))
                vpu_rows.clear()

        done = built = 0
        for i in range(n + LAG):
            if i < n:
                u, t, j = rounds[i]
                h = hh * HU + u
                s = _dot(ks[h // 8, j * TK:(j + 1) * TK, :], masked_q(h, t))
                pending.append((i + LAG, u, t, j, weights(u, t, s).astype(BF16)))
                while done < min(len(units), len(units) * (i + 1) // (n - AHEAD)):
                    vpu_unit(i, *units[done])
                    done += 1
                per_head = n // HU
                want = max(0, t * (NK - 1) + j + 1 - BSTART) * (TK // 8) // (per_head - BSTART - BEND)
                while built < u * (TK // 8) + min(want, TK // 8):
                    broadcast_keys(jnp.minimum(h + 1, H - 1), (kb0, kb1)[(u + 1) % 2] if HU > 1 else kb0.at[(hh + 1) % 2],
                                   built - u * (TK // 8))
                    built += 1
            ready = sorted((e for e in pending if e[0] <= i), key=lambda e: e[0])
            pending[:] = [e for e in pending if e[0] > i]
            for _, u, t, j, p in ready:
                hr = head_rows(hh * HU + u)
                o = _dot(vts[hr, j * TK:(j + 1) * TK], p)
                acc[u, t] = acc[u, t] + o if (u, t) in acc else o
                count[u, t] = count.get((u, t), 0) + 1
                if count[u, t] == NK:
                    ots[hr, t * TQ:(t + 1) * TQ] = (
                        acc[u, t] / den[u, t].sum(0, keepdims=True)).astype(BF16)
        assert not pending
        return 0

    def attention_true_max(i, _):
        h, t = i // NT, i % NT
        q = masked_q(h, t)
        hr = head_rows(h)

        def kbody(j, carry):
            m, den, acc = carry
            keys = pl.ds(pl.multiple_of(j * TK, TK), TK)
            s = _dot(ks[h // 8, keys, :], q)
            m_new = jnp.maximum(m, jnp.max(s, axis=0, keepdims=True))
            a = jnp.exp2(m - m_new)
            p = jnp.exp2(s - m_new)
            den = a * den + jnp.sum(p, axis=0, keepdims=True)
            acc = a * acc + _dot(vts[hr, keys], p.astype(BF16))
            return m_new, den, acc

        init = (jnp.full((1, TQ), -jnp.inf, F32), jnp.zeros((1, TQ), F32),
                jnp.zeros((DH, TQ), F32))
        _, den, acc = lax.fori_loop(0, NK, kbody, init)
        ots[hr, rows(t)] = (acc / den).astype(BF16)
        return 0

    @pl.when(no_shift)
    def _():
        lax.fori_loop(0, H // HU, attention_no_shift, 0)

    @pl.when(jnp.logical_not(no_shift))
    def _():
        lax.fori_loop(0, H * NT, attention_true_max, 0)

    wait("wo", "w3", "w4", "gw")

    def weight_sums(i, _):
        n3, n4 = D // 2 // RO, F // 2 // RO
        _strassen_rhs(w3, w3s, i * n3, n3)
        _strassen_rhs(w4, w4s, i * n4, n4)
        return 0

    lax.fori_loop(0, RO, weight_sums, 0)
    hm, hd, hf = TQ // 2, D // 2, F // 2

    def quadrant(t, q):
        return (pl.ds(pl.multiple_of(t * TQ + q // 2 * hm, hm), hm), pl.ds(q % 2 * hd, hd))

    def out_copy(t, q):
        if not SPLIT:
            return pltpu.make_async_copy(obuf.at[rows(t)], out_hbm.at[rows(t)], out_sem.at[t * 4])
        return pltpu.make_async_copy(obuf.at[quadrant(t, q)], out_hbm.at[quadrant(t, q)],
                                     out_sem.at[t * 4 + q])

    def tile(t, _):
        lhs = _strassen_lhs(*[ln2[quadrant(t, q)].astype(F32) for q in range(4)])
        for c0 in range(0, hf, FC):
            cw = min(FC, hf - c0)
            g = {q: _gelu(c) for q, c in _strassen_mul(lhs, w3, w3s, c0, cw)}
            for i, v in enumerate(_strassen_lhs(g[0], g[1], g[2], g[3])):
                acts[i, :, c0:c0 + cw] = v

        r = rows(t)
        a = lax.dot_general(ots[:, r], wo[...], (((0,), (0,)), ((), ())),
                            preferred_element_type=F32)
        gate = jax.nn.sigmoid(jnp.sum(xs[r, :].astype(F32) * gw[...].astype(F32),
                                      axis=-1, keepdims=True))
        gs[...] = jnp.broadcast_to(gate, (TQ, 128))
        x1 = x1s[r, :]
        x1s[r, :] = x1 + jnp.tile(gs[...], (1, D // 128)) * (a - x1)

        for q, c in _strassen_mul(acts, w4, w4s, 0, hd):
            rest = 1.0 - gs[q // 2 * hm:(q // 2 + 1) * hm, :]
            obuf[quadrant(t, q)] = (
                x1s[quadrant(t, q)] + jnp.tile(rest, (1, hd // 128)) * c).astype(obuf.dtype)
            if SPLIT:
                out_copy(t, q).start()
        if not SPLIT:
            out_copy(t, 0).start()
        return 0

    lax.fori_loop(0, NT, tile, 0)
    for t in range(NT):
        for q in range(4 if SPLIT else 1):
            out_copy(t, q).wait()


@jax.jit
def pallas_gated_mix__mha_block__mixer_s_mlp__prompt_kernel(
    A_x: jax.Array,
    A_wqkv: jax.Array,
    A_wo: jax.Array,
    B_x: jax.Array,
    B_w1: jax.Array,
    B_w2: jax.Array,
    B_w3: jax.Array,
    B_w4: jax.Array,
    gate_w: jax.Array,
):
    hbm = pl.BlockSpec(memory_space=pl.ANY)
    out = pl.pallas_call(
        _kernel,
        in_specs=[hbm] * 8,
        out_specs=hbm,
        out_shape=jax.ShapeDtypeStruct((S, D), A_x.dtype),
        scratch_shapes=[
            pltpu.VMEM((S, D), BF16),
            pltpu.VMEM((D, 3 * D), BF16),
            pltpu.VMEM((3 * D, D), BF16),
            pltpu.VMEM((D, D), BF16),
            pltpu.VMEM((D, D), BF16),
            pltpu.VMEM((D, D), BF16),
            pltpu.VMEM((D, F), BF16),
            pltpu.VMEM((F, D), BF16),
            pltpu.VMEM((5, D // 2, F // 2), BF16),
            pltpu.VMEM((5, F // 2, D // 2), BF16),
            pltpu.VMEM((S + 2 * HALO, D), F32),
            pltpu.VMEM((S, D), F32),
            pltpu.VMEM((S, D), BF16),
            pltpu.VMEM((7, TQ // 2, F // 2), BF16),
            pltpu.VMEM((TQ, 128), F32),
            pltpu.VMEM((D // 128, S, 128), BF16),
            pltpu.VMEM((D // 128, TK, 128), F32),
            pltpu.VMEM((D, S), BF16),
            pltpu.VMEM((D, S), F32),
            pltpu.VMEM((D, S), BF16),
            pltpu.VMEM((D, S), BF16),
            pltpu.VMEM((S, D), A_x.dtype),
            pltpu.VMEM((HU, DH, 8, S + 128 * QP), F32), pltpu.VMEM((PK + 1, 8, 128), F32),
            pltpu.VMEM((DH, TK, 128), F32),
            pltpu.VMEM((P1 + 1, 8, 128), F32),
            pltpu.VMEM((DH, TK, 128), F32),
            pltpu.VMEM((P2 + 1, 8, 128), F32),
            pltpu.VMEM((1, D), BF16),
            pltpu.SemaphoreType.DMA((9 + NT,)),
            pltpu.SemaphoreType.DMA((4 * NT,)),
        ],
        compiler_params=pltpu.CompilerParams(vmem_limit_bytes=100 * 2 ** 20),
    )(A_x.reshape(S, D), A_wqkv, A_wo, B_w1, B_w2, B_w3, B_w4, gate_w.reshape(1, D))
    return out.reshape(A_x.shape)
```

```python
import functools
import math

import jax
import jax.numpy as jnp
from jax import lax
import jax.experimental.pallas as pl
import jax.experimental.pallas.tpu as pltpu

S, D, H, F = 2048, 512, 32, 1792
DH = D // H
TQ = 512
NT = S // TQ
TK = 128
NK = S // TK
HU = 2
LAG = 2
VPU_LAG = 1
KB_START = 4
FC = 128
HALO = 8
Q_SCALE = (DH ** -0.5) * math.log2(math.e)
SCORE_MAX = 40.0
V_MIN, V_MAX = 2.0 ** -60, 2.0 ** 60

BF16 = jnp.bfloat16
F32 = jnp.float32


def _dot(a, b):
    return jnp.dot(a, b, preferred_element_type=F32)


def _layernorm(x):
    m = jnp.mean(x, axis=-1, keepdims=True)
    c = x - m
    v = jnp.mean(c * c, axis=-1, keepdims=True)
    return c * lax.rsqrt(v + 1e-5)


def _gelu(x):
    a = math.sqrt(2.0 / math.pi)
    hx = 0.5 * x
    return hx + hx * jnp.tanh(x * (a + (a * 0.044715) * (x * x)))


def _lane_tile_max(t):
    return functools.reduce(jnp.maximum, [t[:, j:j + 128] for j in range(0, t.shape[1], 128)])


def _max_head_norm2(t):
    sq = t * t
    out = None
    for h in range(H):
        p = sq[h * DH:h * DH + 8] + sq[h * DH + 8:(h + 1) * DH]
        p = p + pltpu.roll(p, 4, 0)
        p = p + pltpu.roll(p, 2, 0)
        p = p + pltpu.roll(p, 1, 0)
        out = p if out is None else jnp.maximum(out, p)
    return _lane_tile_max(out)


def _strassen_lhs(a11, a12, a21, a22):
    return [v.astype(BF16) for v in
            (a11 + a22, a21 + a22, a11, a22, a11 + a12, a21 - a11, a12 - a22)]


def _strassen_rhs(w, ws, r0, m):
    k, n = w.shape[0] // 2, w.shape[1] // 2
    b11, b12, b21, b22 = [
        w[pl.ds(pl.multiple_of(i * k + r0, 16), m), j * n:(j + 1) * n].astype(F32)
        for i in (0, 1) for j in (0, 1)]
    for i, v in enumerate((b11 + b22, b12 - b22, b21 - b11, b11 + b12, b21 + b22)):
        ws[i, pl.ds(pl.multiple_of(r0, 16), m), :] = v.astype(BF16)


def _strassen_mul(lhs, w, ws, c0, cw):
    k, n = w.shape[0] // 2, w.shape[1] // 2
    cols = slice(c0, c0 + cw)
    m2 = _dot(lhs[1], w[:k, cols])
    m4 = _dot(lhs[3], ws[2, :, cols])
    yield 2, m2 + m4
    m5 = _dot(lhs[4], w[k:, n + c0:n + c0 + cw])
    m3 = _dot(lhs[2], ws[1, :, cols])
    yield 1, m3 + m5
    m1 = _dot(lhs[0], ws[0, :, cols])
    m7 = _dot(lhs[6], ws[4, :, cols])
    yield 0, m1 + m4 - m5 + m7
    m6 = _dot(lhs[5], ws[3, :, cols])
    yield 3, m1 - m2 + m3 + m6


def _kernel(x_hbm, wqkv_hbm, wo_hbm, w1_hbm, w2_hbm, w3_hbm, w4_hbm, gw_hbm,
            out_hbm,
            xs, wqkv, wt, wo, w1, w2, w3, w4, w3s, w4s,
            hbuf, x1s, ln2, acts, gs, ks, kf, qts, qf, vts, ots, obuf,
            qb, kb0, kb1, gw, in_sem, out_sem):
    def rows(c):
        return pl.ds(c * TQ if isinstance(c, int) else pl.multiple_of(c * TQ, TQ), TQ)

    def head_rows(h):
        return pl.ds(pl.multiple_of(h * DH, DH), DH)

    def group_rows(h):
        return pl.ds(pl.multiple_of(h // 8 * 128, 128), 128)

    pairs = {"w1": (w1_hbm, w1), "w2": (w2_hbm, w2), "wo": (wo_hbm, wo), "w3": (w3_hbm, w3),
             "w4": (w4_hbm, w4), "gw": (gw_hbm, gw)}
    for i in range(3):
        pairs["w" + "qkv"[i]] = (wqkv_hbm.at[:, pl.ds(i * D, D)], wqkv.at[:, pl.ds(i * D, D)])
    for c in range(NT):
        pairs["x%d" % c] = (x_hbm.at[rows(c)], xs.at[rows(c)])
    copies = {name: pltpu.make_async_copy(src, dst, in_sem.at[i])
              for i, (name, (src, dst)) in enumerate(pairs.items())}

    def start(*names):
        for n in names:
            copies[n].start()

    def wait(*names):
        for n in names:
            copies[n].wait()

    def ln1(c):
        return _layernorm(xs[rows(c), :].astype(F32)).astype(BF16)

    def token_proj(c, xn):
        hbuf[pl.ds(HALO + c * TQ, TQ), :] = _gelu(_dot(xn, w1[...]))

    def token_mix(c):
        cw = D // 4
        hs = jnp.concatenate([
            hbuf[pl.ds(HALO + c * TQ + off, TQ), g * cw:(g + 1) * cw]
            for g, off in enumerate((-1, 1, -2, 2))], axis=-1).astype(BF16)
        x1 = xs[rows(c), :].astype(F32) + _dot(hs, w2[...])
        x1s[rows(c), :] = x1
        ln2[rows(c), :] = _layernorm(x1).astype(BF16)

    stats = {}

    def track(name, m):
        stats[name] = jnp.maximum(stats[name], m) if name in stats else m

    def transpose_w(i):
        wt[i * D:(i + 1) * D, :] = wqkv[:, i * D:(i + 1) * D].T

    def project(c, which):
        for name in which:
            i = "qkv".index(name)
            t = _dot(wt[i * D:(i + 1) * D, :], xs[rows(c), :].T)
            if name == "k":
                kk = t.T.astype(BF16)
                for g in range(D // 128):
                    ks[g, rows(c), :] = kk[:, g * 128:(g + 1) * 128]
                    if c == NT - 1:
                        kf[g] = kk[TQ - TK:, g * 128:(g + 1) * 128].astype(F32)
                track("k", _max_head_norm2(t))
            elif name == "q":
                t = t * Q_SCALE
                qts[:, rows(c)] = t.astype(BF16)
                qf[:, rows(c)] = t
                track("q", _max_head_norm2(t))
            else:
                vts[:, rows(c)] = t.astype(BF16)
                track("v", _lane_tile_max(jnp.abs(t)))

    aligned = {}

    def broadcast_keys(h, dst, d):
        if d == 0:
            aligned["k"] = pltpu.roll(kf[h // 8], (128 - (h % 8) * DH) % 128, 1)
        dst[d] = jnp.broadcast_to(aligned["k"][:, d:d + 1], (TK, 128))

    start("x0", "wk")
    hbuf[0:HALO, :] = jnp.zeros((HALO, D), F32)
    hbuf[HALO + S:, :] = jnp.zeros((HALO, D), F32)
    wait("x0")
    start("w1", "wq")
    xn0 = ln1(0)
    wait("wk")
    start("wv", "x1")
    transpose_w(1)
    project(0, "k")
    wait("w1", "wq")
    start("x2", "x3", "w2")
    token_proj(0, xn0)
    transpose_w(0)
    project(0, "q")
    wait("wv", "x1")
    transpose_w(2)
    project(1, "k")
    token_proj(1, ln1(1))
    project(0, "v")
    wait("x2", "x3", "w2")
    start("wo", "w3", "w4", "gw")
    project(1, "q")
    token_proj(2, ln1(2))
    token_mix(0)
    project(2, "kq")
    token_proj(3, ln1(3))
    token_mix(1)
    project(3, "kq")
    token_mix(2)
    project(1, "v")
    token_mix(3)
    for d in range(DH):
        broadcast_keys(0, kb0, d)
    project(2, "v")
    project(3, "v")

    vm = jnp.max(stats["v"], axis=1, keepdims=True)
    v_ok = jnp.logical_or(vm == 0.0, jnp.logical_and(vm >= V_MIN, vm <= V_MAX))
    v_bad = jnp.max(jnp.where(v_ok, 0.0, 1.0), axis=0, keepdims=True)
    bound2 = (jnp.max(stats["q"], axis=1, keepdims=True)
              * jnp.max(stats["k"], axis=1, keepdims=True) * 1.02)
    safe = jnp.where(bound2 <= SCORE_MAX * SCORE_MAX, 1.0 - v_bad, 0.0)
    no_shift = jnp.min(safe) > 0.5

    head_of_row = lax.broadcasted_iota(jnp.int32, (128, TQ), 0) // DH

    def masked_q(h, c):
        q = qts[group_rows(h), c].astype(F32)
        return jnp.where(head_of_row == h % 8, q, 0.0).astype(BF16)

    def attention_no_shift(hh, _):
        rounds = [(u, t, j) for u in range(HU) for t in range(NT) for j in range(NK - 1)]
        units = [(u, t, r) for u in range(HU) for t in range(NT) for r in range(TK // 8)]
        n = len(rounds)
        per_head = n // HU
        kbs = (kb0, kb1)
        pending, acc, den, count, vpu_rows = [], {}, {}, {}, []

        def cols(t):
            return slice(t * TQ, (t + 1) * TQ)

        def weights(u, t, s):
            p = jnp.exp2(s)
            tot = p.reshape(-1, 8, TQ).sum(0)
            den[u, t] = den[u, t] + tot if (u, t) in den else tot
            return p

        def vpu_unit(i, u, t, r):
            if (t, r) == (0, 0):
                q = qf[head_rows(hh * HU + u), :]
                for d in range(DH):
                    qb[u, d] = jnp.broadcast_to(q[d:d + 1, :], (8, S))
            s = functools.reduce(jnp.add, [
                jnp.tile(kbs[u % 2][d, r * 8:(r + 1) * 8, :], (1, TQ // 128)) * qb[u, d, :, cols(t)]
                for d in range(DH)])
            vpu_rows.append(weights(u, t, s))
            if r == TK // 8 - 1:
                pending.append((i + VPU_LAG, u, t, NK - 1,
                                jnp.concatenate(vpu_rows, 0).astype(BF16)))
                vpu_rows.clear()

        done = built = 0
        for i in range(n + LAG):
            if i < n:
                u, t, j = rounds[i]
                h = hh * HU + u
                s = _dot(ks[h // 8, j * TK:(j + 1) * TK, :], masked_q(h, cols(t)))
                pending.append((i + LAG, u, t, j, weights(u, t, s).astype(BF16)))
                while done < min(len(units), len(units) * (i + 1) // (n - 1)):
                    vpu_unit(i, *units[done])
                    done += 1
                want = max(0, i % per_head + 1 - KB_START) * DH // (per_head - KB_START)
                while built < u * DH + want:
                    broadcast_keys(jnp.minimum(h + 1, H - 1), kbs[(u + 1) % 2], built - u * DH)
                    built += 1
            ready = sorted((e for e in pending if e[0] <= i), key=lambda e: e[0])
            pending[:] = [e for e in pending if e[0] > i]
            for _, u, t, j, p in ready:
                hr = head_rows(hh * HU + u)
                o = _dot(vts[hr, j * TK:(j + 1) * TK], p)
                acc[u, t] = acc[u, t] + o if (u, t) in acc else o
                count[u, t] = count.get((u, t), 0) + 1
                if count[u, t] == NK:
                    ots[hr, cols(t)] = (
                        acc[u, t] / den[u, t].sum(0, keepdims=True)).astype(BF16)
        assert not pending
        return 0

    def attention_true_max(i, _):
        h, t = i // NT, i % NT
        q = masked_q(h, rows(t))
        hr = head_rows(h)

        def kbody(j, carry):
            m, den, acc = carry
            keys = pl.ds(pl.multiple_of(j * TK, TK), TK)
            s = _dot(ks[h // 8, keys, :], q)
            m_new = jnp.maximum(m, jnp.max(s, axis=0, keepdims=True))
            a = jnp.exp2(m - m_new)
            p = jnp.exp2(s - m_new)
            den = a * den + jnp.sum(p, axis=0, keepdims=True)
            acc = a * acc + _dot(vts[hr, keys], p.astype(BF16))
            return m_new, den, acc

        init = (jnp.full((1, TQ), -jnp.inf, F32), jnp.zeros((1, TQ), F32),
                jnp.zeros((DH, TQ), F32))
        _, den, acc = lax.fori_loop(0, NK, kbody, init)
        ots[hr, rows(t)] = (acc / den).astype(BF16)
        return 0

    @pl.when(no_shift)
    def _():
        lax.fori_loop(0, H // HU, attention_no_shift, 0)

    @pl.when(jnp.logical_not(no_shift))
    def _():
        lax.fori_loop(0, H * NT, attention_true_max, 0)

    wait("wo", "w3", "w4", "gw")

    def weight_sums(i, _):
        _strassen_rhs(w3, w3s, i * 16, 16)
        _strassen_rhs(w4, w4s, jnp.minimum(i, F // 2 // 64 - 1) * 64, 64)
        return 0

    lax.fori_loop(0, D // 2 // 16, weight_sums, 0)
    hm, hd, hf = TQ // 2, D // 2, F // 2

    def quadrant(t, q):
        return (pl.ds(pl.multiple_of(t * TQ + q // 2 * hm, hm), hm), pl.ds(q % 2 * hd, hd))

    def out_copy(t, q):
        return pltpu.make_async_copy(obuf.at[quadrant(t, q)], out_hbm.at[quadrant(t, q)],
                                     out_sem.at[t * 4 + q])

    def tile(t, _):
        lhs = _strassen_lhs(*[ln2[quadrant(t, q)].astype(F32) for q in range(4)])
        for c0 in range(0, hf, FC):
            cw = min(FC, hf - c0)
            g = {q: _gelu(c) for q, c in _strassen_mul(lhs, w3, w3s, c0, cw)}
            for i, v in enumerate(_strassen_lhs(g[0], g[1], g[2], g[3])):
                acts[i, :, c0:c0 + cw] = v

        r = rows(t)
        a = lax.dot_general(ots[:, r], wo[...], (((0,), (0,)), ((), ())),
                            preferred_element_type=F32)
        gate = jax.nn.sigmoid(jnp.sum(xs[r, :].astype(F32) * gw[...].astype(F32).reshape(1, D),
                                      axis=-1, keepdims=True))
        gs[...] = jnp.broadcast_to(gate, (TQ, 128))
        x1 = x1s[r, :]
        x1s[r, :] = x1 + jnp.tile(gs[...], (1, D // 128)) * (a - x1)

        for q, c in _strassen_mul(acts, w4, w4s, 0, hd):
            rest = 1.0 - gs[q // 2 * hm:(q // 2 + 1) * hm, :]
            obuf[quadrant(t, q)] = (
                x1s[quadrant(t, q)] + jnp.tile(rest, (1, hd // 128)) * c).astype(obuf.dtype)
            out_copy(t, q).start()
        return 0

    lax.fori_loop(0, NT, tile, 0)
    for t in range(NT):
        for q in range(4):
            out_copy(t, q).wait()


@jax.jit
def pallas_gated_mix__mha_block__mixer_s_mlp__prompt_kernel(
    A_x: jax.Array,
    A_wqkv: jax.Array,
    A_wo: jax.Array,
    B_x: jax.Array,
    B_w1: jax.Array,
    B_w2: jax.Array,
    B_w3: jax.Array,
    B_w4: jax.Array,
    gate_w: jax.Array,
):
    hbm = pl.BlockSpec(memory_space=pl.ANY)
    out = pl.pallas_call(
        _kernel,
        in_specs=[hbm] * 8,
        out_specs=hbm,
        out_shape=jax.ShapeDtypeStruct((S, D), A_x.dtype),
        scratch_shapes=[
            pltpu.VMEM((S, D), BF16),
            pltpu.VMEM((D, 3 * D), BF16),
            pltpu.VMEM((3 * D, D), BF16),
            pltpu.VMEM((D, D), BF16),
            pltpu.VMEM((D, D), BF16),
            pltpu.VMEM((D, D), BF16),
            pltpu.VMEM((D, F), BF16),
            pltpu.VMEM((F, D), BF16),
            pltpu.VMEM((5, D // 2, F // 2), BF16),
            pltpu.VMEM((5, F // 2, D // 2), BF16),
            pltpu.VMEM((S + 2 * HALO, D), F32),
            pltpu.VMEM((S, D), F32),
            pltpu.VMEM((S, D), BF16),
            pltpu.VMEM((7, TQ // 2, F // 2), BF16),
            pltpu.VMEM((TQ, 128), F32),
            pltpu.VMEM((D // 128, S, 128), BF16),
            pltpu.VMEM((D // 128, TK, 128), F32),
            pltpu.VMEM((D, S), BF16),
            pltpu.VMEM((D, S), F32),
            pltpu.VMEM((D, S), BF16),
            pltpu.VMEM((D, S), BF16),
            pltpu.VMEM((S, D), A_x.dtype),
            pltpu.VMEM((HU, DH, 8, S), F32),
            pltpu.VMEM((DH, TK, 128), F32),
            pltpu.VMEM((DH, TK, 128), F32),
            pltpu.VMEM((D,), BF16),
            pltpu.SemaphoreType.DMA((9 + NT,)),
            pltpu.SemaphoreType.DMA((4 * NT,)),
        ],
        compiler_params=pltpu.CompilerParams(vmem_limit_bytes=100 * 2 ** 20),
    )(A_x.reshape(S, D), A_wqkv, A_wo, B_w1, B_w2, B_w3, B_w4, gate_w)
    return out.reshape(A_x.shape)
```
